```python
import os as _os
_os.environ.setdefault("JAX_PLATFORMS", "cpu")
import jax
import jax.numpy as jnp

def _softmax(x, axis=-1):
    return jax.nn.softmax(x, axis=axis)
def _gelu(x):
    return jax.nn.gelu(x, approximate=True)
def _silu(x):
    return jax.nn.silu(x)
def _sigmoid(x):
    return jax.nn.sigmoid(x)
def _layernorm(x, axis=-1, eps=1e-5):
    m = jnp.mean(x, axis=axis, keepdims=True)
    v = jnp.var(x, axis=axis, keepdims=True)
    return (x - m) / jnp.sqrt(v + eps)
def _scatter_add(tgt, idx, src, axis=0):
    return tgt.at[idx].add(src)
def _segment_sum(src, seg, n):
    return jax.ops.segment_sum(src, seg, n)
class _Rng:
    def __init__(self, key):
        self._k = key
    def _next(self):
        self._k, sub = jax.random.split(self._k)
        return sub
    def normal(self, shape):
        return jax.random.normal(self._next(), shape, dtype=jnp.bfloat16)
    def randint(self, lo, hi, shape):
        return jax.random.randint(self._next(), shape, lo, hi, dtype=jnp.int32)
    def uniform(self, shape, lo=0.0, hi=1.0):
        return jax.random.uniform(self._next(), shape, jnp.bfloat16, lo, hi)
    def permutation(self, n):
        return jax.random.permutation(self._next(), n)


kernel_name = 'sequential_preLN__sliding_local_dilated__dense_activation_silu__prompt'

def setup_inputs():
    _rng = _Rng(jax.random.key(int.from_bytes(__import__("os").urandom(4), "little")))
    _w = (lambda a: (lambda t: t.astype(jnp.bfloat16) if jnp.issubdtype(t.dtype, jnp.floating) else t)(jnp.asarray(a)))
    def _A_setup():
        B, S, D = 1, 2048, 1024
        return {
            "x": _w((lambda *s: _rng.normal(s) * 0.05)(B, S, D)),
            "wqkv": _w((lambda *s: _rng.normal(s) * 0.05)(D, 3 * D)),
            "wo": _w((lambda *s: _rng.normal(s) * 0.05)(D, D)),
        }
    _A_in = _A_setup()

    def _B_setup():
        B, S, D, F = 1, 2048, 1024, 3584
        return {
            "x": _w((lambda *s: _rng.normal(s) * 0.05)(B, S, D)),
            "w1": _w((lambda *s: _rng.normal(s) * 0.05)(D, F) * (D ** -0.5)),
            "w2": _w((lambda *s: _rng.normal(s) * 0.05)(F, D) * (F ** -0.5)),
        }
    _B_in = _B_setup()

    return {
        "A_x": _A_in["x"],
        "A_wqkv": _A_in["wqkv"],
        "A_wo": _A_in["wo"],
        "B_x": _B_in["x"],
        "B_w1": _B_in["w1"],
        "B_w2": _B_in["w2"],
    }

def reference(A_x, A_wqkv, A_wo, B_x, B_w1, B_w2):
    def _A_ref(x, wqkv, wo):
        B, S, D = x.shape
        H = 32; Dh = D // H
        W, dil = 8, 2
        qkv = (lambda x, *d: x.transpose(*d))((x @ wqkv).reshape(B, S, 3, H, Dh), 2, 0, 3, 1, 4)
        q, k, v = qkv[0], qkv[1], qkv[2]
        scale = Dh ** -0.5
        pos = jnp.arange(S)
        off = jnp.arange(W) * dil
        idx = pos[:, None] - off[None, :]
        mask = idx >= 0
        idx_c = jnp.where(mask, idx, 0).reshape(-1)
        kg = k[:, :, idx_c, :].reshape(B, H, S, W, Dh)
        vg = v[:, :, idx_c, :].reshape(B, H, S, W, Dh)
        logits = jnp.einsum("bhsd,bhswd->bhsw", q, kg) * scale
        logits = jnp.where(mask[None, None, :, :], logits, -1e9)
        attn = _softmax(logits, axis=-1)
        o = jnp.einsum("bhsw,bhswd->bhsd", attn, vg)
        return (lambda x, *d: x.transpose(*d))(o, 0, 2, 1, 3).reshape(B, S, D) @ wo

    def _B_ref(x, w1, w2):
        h = jnp.einsum("bsd,df->bsf", x, w1)
        h = _silu(h)
        out = jnp.einsum("bsf,fd->bsd", h, w2)
        return out

    x = A_x
    h = x + _A_ref(_layernorm(x, axis=-1), A_wqkv, A_wo)
    h2 = h + _B_ref(_layernorm(h, axis=-1), B_w1, B_w2)
    return h2
```

```python
import functools
import math
import operator

import jax
import jax.numpy as jnp
import jax.experimental.pallas as pl
import jax.experimental.pallas.tpu as pltpu

F32, BF16, U32, I32 = jnp.float32, jnp.bfloat16, jnp.uint32, jnp.int32

S, D, F = 2048, 1024, 3584
DH, WIN, DIL = 32, 8, 2
LANE = 128
NL = D // LANE
HALO = 16
EPS = 1e-5
LOG2E = math.log2(math.e)

TM = 256
NT = S // TM
RA = TM // 2
RO = TM // 4
RB = TM // 4
FC = 512
NC = F // FC
QPARTS = 4
SHARE = 3
N_PROJ = 4 * 7

ORDER_PROJ = (5, 2, 4, 0, 1, 3, 6)
ORDER_LAST = (5, 1, 3, 0, 2, 4, 6)
ORDER_UP = (6, 4, 2, 0, 3, 1, 5), (1, 3, 0, 6, 4, 2, 5)
ORDER_DOWN = (2, 4, 1, 3, 0, 5, 6), (2, 4, 1, 3, 0, 5, 6)


def _add(x, y):
    return [p + q for p, q in zip(x, y)]


def _sub(x, y):
    return [p - q for p, q in zip(x, y)]


def lhs_term(i, a11, a12, a21, a22):
    return (
        lambda: _add(a11, a22), lambda: _add(a21, a22), lambda: a11, lambda: a22,
        lambda: _add(a11, a12), lambda: _sub(a21, a11), lambda: _sub(a12, a22),
    )[i]()


def rhs_term(i, b11, b12, b21, b22):
    return (
        lambda: _add(b11, b22), lambda: b11, lambda: _sub(b12, b22), lambda: _sub(b21, b11),
        lambda: b22, lambda: _add(b11, b12), lambda: _add(b21, b22),
    )[i]()


RHS_BLOCKS = ((0, 3), (0,), (1, 3), (2, 0), (3,), (0, 1), (2, 3))
OUTPUTS = ({0: 1, 3: 1, 4: -1, 6: 1}, {2: 1, 4: 1}, {1: 1, 3: 1}, {0: 1, 1: -1, 2: 1, 5: 1})


def combine(product, emit, order):
    acc = [None] * 4
    left = [len(out) for out in OUTPUTS]
    for i in order:
        m = yield from product(i)
        for k, out in enumerate(OUTPUTS):
            if i in out:
                if acc[k] is None:
                    acc[k] = m, out[i]
                elif acc[k][1] < 0:
                    acc[k] = _sub(m, acc[k][0]), 1
                else:
                    acc[k] = (_add if out[i] > 0 else _sub)(acc[k][0], m), 1
                left[k] -= 1
                if not left[k]:
                    emit(k, acc[k][0])


def combine2(leaf, emit, orders):
    def outer(i):
        res = [None] * 4

        def keep(k, c):
            res[k] = c[0]
        yield from combine(lambda j: leaf(7 * i + j), keep, orders[1])
        return res

    def emit_outer(ko, cs):
        for ki in range(4):
            emit(2 * (ko // 2) + ki // 2, 2 * (ko % 2) + ki % 2, cs[ki])
    yield from combine(outer, emit_outer, orders[0])


def lhs_terms2(blk, i):
    outer = []
    for hi_r in range(2):
        for hi_c in range(2):
            flat = []
            for lo_r in range(2):
                for lo_c in range(2):
                    flat += blk[2 * hi_r + lo_r][2 * hi_c + lo_c]
            outer.append(flat)
    o = lhs_term(i, *outer)
    n = len(o) // 4
    inner = [o[q * n:(q + 1) * n] for q in range(4)]
    return [lhs_term(j, *inner) for j in range(7)]


def pack(lo, hi):
    return pltpu.bitcast(pltpu.pack_elementwise([lo, hi], packed_dtype=BF16), U32)


def unpack(w):
    return [pltpu.unpack_elementwise(w, index=i, packed_dtype=BF16, unpacked_dtype=F32)
            for i in range(2)]


def as_bf16(w):
    return pltpu.bitcast(w, BF16)


def mm(a, b):
    return jnp.dot(a, b, preferred_element_type=F32)


def total(xs):
    return functools.reduce(operator.add, xs)


def lane_mean(part):
    return jnp.sum(part, axis=1, keepdims=True) * (1.0 / D)


def aligned(start, size):
    return pl.ds(start if isinstance(start, int) else pl.multiple_of(start, size), size)


def lanes(j, n=1):
    return slice(j * LANE, (j + n) * LANE)


def chain(*gens):
    for g in gens:
        yield from g


def run(main, n_main, side=(), lo=0.0, hi=1.0):
    done = step = 0
    for _ in main:
        step += 1
        want = min(len(side), math.ceil((step / n_main - lo) / (hi - lo) * len(side)))
        while done < want:
            side[done]()
            done += 1
    assert step == n_main and done == len(side)


class Pacer:
    def __init__(self, width):
        self.state = [jnp.full((8, LANE), k, U32) for k in range(width)]
        self.count = 0

    def tick(self, piece=None):
        def thunk():
            k = self.count % len(self.state)
            self.count += 1
            v = self.state[k]
            if piece is not None:
                v = v ^ pltpu.bitcast(piece(), U32)
            self.state[k] = pltpu.roll(v, 1, 1)
        return thunk

    def finish(self, sink, tail):
        out = []
        for j in range(len(self.state)):
            x = pltpu.bitcast(self.state[(self.count - 1 - j) % len(self.state)], F32)
            for _ in range(j * tail):
                x = jnp.tanh(x)
            out.append(x)
        sink[...] = total(out)


def kernel(x_hbm, wqkv_hbm, wo_hbm, w1_hbm, w2_hbm, out_hbm,
           xb, wqkv_raw, wo_raw, w1_raw, w2_raw,
           wqkv_c, wo_c, w1_c, w2_c,
           a1, qkv, new, ob, o_c,
           hb, stats, zb, a2, sink, zero, sem_x, sem_w, sem_1, sem_2, sem_y):
    for k in range(8):
        zero[k] = 0

    def tile_rows(t, off, n, stride=1):
        base = t * TM if isinstance(t, int) else pl.multiple_of(t * TM, TM)
        return pl.ds(base + off, n, stride=stride)

    def cp_x(t):
        rows = tile_rows(t, 0, TM)
        return pltpu.make_async_copy(x_hbm.at[rows], xb.at[rows], sem_x.at[t])

    def cp_qkv(m):
        src, dst = (r.at[:, :, aligned(m * D, D)] for r in (wqkv_hbm, wqkv_raw))
        return pltpu.make_async_copy(src, dst, sem_w.at[m])

    def cp_q(part):
        n = D // 2 // QPARTS
        src, dst = (r.at[:, aligned(part * n, n), pl.ds(0, D)] for r in (wqkv_hbm, wqkv_raw))
        return pltpu.make_async_copy(src, dst, sem_w.at[3 + part])

    def cp_wo():
        return pltpu.make_async_copy(wo_hbm, wo_raw, sem_w.at[0])

    def cp_w1(c):
        return pltpu.make_async_copy(w1_hbm.at[:, aligned(c * FC, FC)], w1_raw.at[c], sem_1.at[c])

    def cp_w2(c):
        return pltpu.make_async_copy(w2_hbm.at[aligned(c * FC, FC)], w2_raw.at[c], sem_2.at[c])

    def cp_y(t, n, rh):
        src, dst = (r.at[tile_rows(t, rh * TM // 2, TM // 2), pl.ds(n * D // 2, D // 2)]
                    for r in (xb, out_hbm))
        return pltpu.make_async_copy(src, dst, sem_y.at[4 * t + 2 * n + rh])

    def reorder_columns(groups):
        l = jax.lax.broadcasted_iota(I32, (8, LANE), 1)
        groups = [[g[-t % NL] for t in range(NL)] for g in groups]
        for b in (1, 2, 4):
            move = (l & b) != 0
            groups = [[jnp.where(move, g[(t - b) % NL], g[t]) for t in range(NL)] for g in groups]
        e = l >> 5
        a = (l >> 1) & 3
        j = ((l >> 3) & 1) | ((l & 1) << 1) | (((l >> 4) & 1) << 2)
        out = [[None] * NL for _ in groups]
        for t in range(NL):
            for k, g in enumerate(groups):
                out[k][t] = jnp.take_along_axis(g[t], 32 * a + 8 * e + ((j + t) & 7), axis=1)
        return out

    def qkv_slab(m, i, half):
        w = pltpu.bitcast(wqkv_raw[half, aligned(16 * i, 16), aligned(m * D, D)], U32)
        return [w[:, lanes(j)] for j in range(NL)]

    def qkv_sums(m, i, top, bottom):
        for t in range(4):
            raw = (top[t], top[t + 4], bottom[t], bottom[t + 4])
            blk = [unpack(w) for w in raw]
            for p in range(7):
                w = raw[0] if p == 1 else raw[3] if p == 4 else pack(*rhs_term(p, *blk))
                wqkv_c[m, t * 7 + p, aligned(8 * i, 8), :] = w

    def prep_qkv(m):
        held = {}

        def reorder(i, half):
            held[half], = reorder_columns([qkv_slab(m, i, half)])
        return [w for i in range(D // 32) for w in (
            functools.partial(reorder, i, 0), functools.partial(reorder, i, 1),
            lambda i=i: qkv_sums(m, i, held[0], held[1]))]

    def prep_wo():
        def staged(e, j, a):
            return 9 * (32 * e + 8 * (j >> 1) + 4 * (j & 1) + a)

        def widen(i):
            j, a = i // 4, i % 4
            seen = []
            for n in range(NL):
                w = wo_raw[32 * i:32 * (i + 1), lanes(n)].astype(F32)
                for e in range(4):
                    g = w[8 * e:8 * e + 8]
                    hb[n, pl.ds(staged(e, j, a), 8), :] = pltpu.roll(g, 8 - j, 0) if j else g
                seen.append(g)
            return total(seen)

        def rows(n, t, e, j_hi):
            return [hb[n, pl.ds(staged(e, 4 * j_hi + 2 * j_mid, 0) + t, 8, stride=9), :]
                    for j_mid in range(2)]

        def sums(n, t, e):
            seen = []
            for j_hi in range(2):
                blk = [rows(n, t, e, j_hi), rows(n + 4, t, e, j_hi),
                       rows(n, t + 4, e, j_hi), rows(n + 4, t + 4, e, j_hi)]
                r = 64 * t + 16 * e + 8 * j_hi
                words = [pack(*rhs_term(p, *blk)) for p in range(7)]
                for p in range(7):
                    wo_c[n * 7 + p, r:r + 8, :] = words[p]
                seen.append(words[5] ^ words[6])
            return seen[0] ^ seen[1]

        return ([functools.partial(widen, i) for i in range(D // 32)]
                + [functools.partial(sums, n, t, e)
                   for n in range(4) for t in range(4) for e in range(4)])

    def prep_ffn(step):
        groups = ((1, 5), (2, 4, 0), (3, 6))

        def piece(load, store, group):
            held = {}

            def block(q):
                if q not in held:
                    held[q] = [x for r in range(2) for c in range(2)
                               for x in unpack(load(2 * (q // 2) + r, 2 * (q % 2) + c))]
                return held[q]
            for p in group:
                o = rhs_term(p, *[block(q) if q in RHS_BLOCKS[p] else None for q in range(4)])
                words = [pack(*rhs_term(j, o[0:2], o[2:4], o[4:6], o[6:8])) for j in range(7)]
                for j in range(7):
                    store(p * 7 + j, words[j])
            return words[2] ^ words[3]

        def up(c, i, n):
            def load(r, b):
                rows = aligned(256 * r + 16 * i, 16)
                return pltpu.bitcast(w1_raw[c + zero[n], rows, lanes(b)], U32)

            def store(p, word):
                w1_c[c, p, aligned(8 * i, 8), :] = word
            return piece(load, store, groups[n])

        def down(c, g, n):
            i, half = g >> 1, g & 1

            def load(r, b):
                return pltpu.bitcast(w2_raw[c + zero[n], aligned(128 * r + 16 * i, 16),
                                            aligned((4 * half + b) * LANE, LANE)], U32)

            def store(p, word):
                w2_c[half, p, c, aligned(8 * i, 8), :] = word
            return piece(load, store, groups[n])

        slabs = [(NC - 1, jnp.minimum(SHARE * step + i, 15)) for i in range(SHARE)]
        slabs += [(step, i) for i in range(16)]
        return [functools.partial(f, c, i, n) for c, i in slabs for f in (up, down)
                for n in range(len(groups))]

    def ln1(t, slot):
        mean, inv = {}, {}

        def load(k, rh, i, cols):
            return pltpu.bitcast(xb[tile_rows(t + zero[k], rh * RA + 16 * i, 16), cols], U32)

        def rows_of(k, rh, i):
            w = load(k, rh, i, slice(None))
            return zip(*[unpack(w[:, lanes(j)]) for j in range(NL)])

        def means(rh, i):
            part = [total(x) for x in rows_of(0, rh, i)]
            mean[rh, i] = [lane_mean(p) for p in part]
            return total(part)

        def scales(rh, i):
            part = [total([(u - m) * (u - m) for u in x])
                    for x, m in zip(rows_of(1, rh, i), mean[rh, i])]
            inv[rh, i] = [jax.lax.rsqrt(lane_mean(p) + EPS) for p in part]
            return total(part)

        def sums(i, j):
            blk = [[(u - m) * r for u, m, r in zip(unpack(load(2, rh, i, lanes(j + 4 * kh))),
                                                   mean[rh, i], inv[rh, i])]
                   for rh in range(2) for kh in range(2)]
            words = [pack(*lhs_term(p, *blk)) for p in range(7)]
            for p in range(7):
                a1[slot, p, 8 * i:8 * i + 8, lanes(j)] = words[p]
            return words[5] ^ words[6]

        groups = [(rh, i) for i in range(RA // 16) for rh in range(2)]
        return ([functools.partial(means, *g) for g in groups],
                [functools.partial(scales, *g) for g in groups],
                [functools.partial(sums, i, j) for i in range(RA // 16) for j in range(4)])

    def project(slot, m, buf, dst, before=None):
        for n in range(4):
            if before:
                before(n)

            def product(p):
                r = mm(as_bf16(a1[slot, p]), as_bf16(wqkv_c[m, n * 7 + p]))
                yield
                return [r]

            def emit(k, c):
                r = HALO + (k // 2) * RA
                buf[dst, n + 4 * (k % 2), r:r + RA, :] = c[0]
            yield from combine(product, emit, ORDER_PROJ)

    def first_halo():
        for j in range(NL):
            qkv[1, j, 0:HALO, :] = jnp.zeros((HALO, LANE), F32)
            qkv[2, j, 0:HALO, :] = jnp.broadcast_to(qkv[2, j, HALO:HALO + 1, :], (HALO, LANE))

    def hand_over(moved_rows):
        def move(m, r, n):
            for j in range(NL):
                qkv[m, j, HALO + r:HALO + r + n, :] = new[m, j, HALO + r:HALO + r + n, :]
            moved_rows[m] += n
            return qkv[m + zero[7], 0, HALO + r:HALO + r + 8, :]
        for m in (1, 2):
            for j in range(NL):
                qkv[m, j, 0:HALO, :] = qkv[m, j, TM:TM + HALO, :]
            move(m, 0, 16)
        return [[functools.partial(move, m, r, 24) for r in range(16, TM, 24)] for m in (1, 2)]

    def attention(buf, first=False, moved=(True,) * 4):
        held = {}

        def window(r, w):
            return pl.ds(HALO + r - DIL * w, 8)

        def score(r, w):
            if w == 0:
                held[r, "q"] = [(buf if moved[j % 4] else new)[0, j, HALO + r:HALO + r + 8, :]
                                for j in range(NL)]
            a = total([held[r, "q"][j] * buf[1, j, window(r, w), :] for j in range(NL)])
            held[r, w] = a + pltpu.roll(a, 64, 1)

        def logit(r, w):
            a = (held[r, w] + pltpu.roll(held[r, w], 32, 1)) * (DH ** -0.5 * LOG2E)
            if first and r < DIL * w:
                pos = r + jax.lax.broadcasted_iota(I32, (8, LANE), 0)
                a = jnp.where(pos >= DIL * w, a, -1e9 * LOG2E)
            held[r, w] = a
            held[r, "max"] = a if w == 0 else jnp.maximum(held[r, "max"], a)

        def softmax(r):
            ex = [jnp.exp2(held[r, w] - held[r, "max"]) for w in range(WIN)]
            inv = 1.0 / total(ex)
            held[r] = [e * inv for e in ex]

        def value(r, j):
            o = total([held[r][w] * buf[2, j, window(r, w), :] for w in range(WIN)])
            ob[r:r + 8, lanes(j)] = o
            return o

        return [([functools.partial(score, r, w) for w in range(WIN)],
                 [functools.partial(logit, r, w) for w in range(WIN)],
                 functools.partial(softmax, r),
                 [functools.partial(value, r, j) for j in range(NL)]) for r in range(0, TM, 8)]

    def attention_work(pace, att, riders=(), lead=True):
        stages = []
        n = len(att)
        placed = [0] * len(riders)
        for u in range(n + 2):
            work = []
            stages.append(work)
            for w in range(WIN):
                if u < n:
                    work.append(att[u][0][w])
                if u >= 2 or lead:
                    work.append(pace.tick(att[u - 2][3][w] if u >= 2 else None))
                if 1 <= u <= n:
                    work.append(att[u - 1][1][w])
                for k, (thunks, lo, hi) in enumerate(riders):
                    want = (WIN * (u - lo) + w + 1) * len(thunks) // (WIN * (hi - lo))
                    want = min(len(thunks), max(0, want))
                    work += thunks[placed[k]:want]
                    placed[k] = want
            if 1 <= u <= n:
                work.append(att[u - 1][2])
        assert placed == [len(thunks) for thunks, _, _ in riders]
        return stages

    def norm_riders(pace, norm, *bounds):
        return [([pace.tick(w) for w in stage], lo, hi)
                for stage, lo, hi in zip(norm, bounds, bounds[1:])]

    def out_sums():
        def unit(s, i):
            blk = []
            for rh in range(2):
                r = (2 * s + rh) * RO + 16 * i
                blk += [[ob[r:r + 16, lanes(4 * kh, 4)]] for kh in range(2)]
            terms = [lhs_term(p, *blk)[0] for p in range(7)]
            for p in range(7):
                r = (s * 7 + p) * RO + 16 * i
                o_c[r:r + 16, :] = terms[p].astype(BF16)
            return terms[5][0:8, lanes(0)] + terms[6][8:16, lanes(3)]
        return [functools.partial(unit, s, i) for s in range(2) for i in range(RO // 16)]

    def out_proj(t, halves, order):
        for s in halves:
            for n in range(4):
                def product(p):
                    r = mm(o_c[(s * 7 + p) * RO:(s * 7 + p + 1) * RO, :], as_bf16(wo_c[n * 7 + p]))
                    yield
                    return [r]

                def emit(k, c):
                    r = tile_rows(t, (2 * s + k // 2) * RO, RO)
                    j = n + 4 * (k % 2)
                    hb[j, r, :] = xb[r, lanes(j)].astype(F32) + c[0]
                yield from combine(product, emit, order)

    def quad_rows(t, rb, i):
        return tile_rows(t, rb * RB + 32 * (i % 2) + i // 2, 8, stride=4)

    def ln2_stats(t):
        def means(rb, i):
            part = total([hb[j, quad_rows(t, rb, i), :] for j in range(NL)])
            stats[0, tile_rows(t, rb * RB + 8 * i, 8), :] = jnp.broadcast_to(lane_mean(part), (8, LANE))
            return part

        def scales(rb, i):
            dst = tile_rows(t, rb * RB + 8 * i, 8)
            mean = stats[0, dst, :]
            cen = [hb[j, quad_rows(t + zero[6], rb, i), :] - mean for j in range(NL)]
            part = total([u * u for u in cen])
            stats[1, dst, :] = jnp.broadcast_to(0.5 * jax.lax.rsqrt(lane_mean(part) + EPS), (8, LANE))
            return part
        return [functools.partial(f, rb, i) for f in (means, scales) for rb in range(4) for i in range(8)]

    def ln2_sums(t):
        z = zero[1]

        def norm(rb, i):
            src = tile_rows(t, rb * RB + 8 * i, 8)
            mean, inv = stats[0, src, :], stats[1, src, :]
            r = rb * RB + 8 * i
            out = [(hb[j, quad_rows(t, rb, i), :] - mean) * inv for j in range(NL)]
            for j in range(NL):
                zb[z, j, r:r + 8, :] = out[j]
            return total(out)

        def sums(i, n, p):
            blk = [[[zb[zero[2 + p % 4], 2 * c + n, pl.ds(rb * RB + 8 * (i + 4 * h), 8), :]
                     for h in range(2)] for c in range(4)] for rb in range(4)]
            words = [pack(*term) for term in lhs_terms2(blk, p)]
            for j in range(7):
                a2[0, p * 7 + j, 8 * i:8 * i + 8, lanes(n)] = words[j]
            return words[5] ^ words[6]

        return ([functools.partial(norm, rb, i + 4 * h)
                 for i in range(4) for rb in range(4) for h in range(2)]
                + [functools.partial(sums, i, n, p)
                   for i in range(4) for n in range(2) for p in range(7)])

    def ffn_step(t, carry):
        g = [[] for _ in range(49)]
        pace = Pacer(2)
        for c in range(NC):
            act = {}

            def leaf(p):
                r = mm(as_bf16(a2[0, p]), as_bf16(w1_c[c, p]))
                yield
                return [r]

            def emit(rb, nb, v):
                act[rb, nb] = v * jnp.tanh(v) + v
            run(combine2(leaf, emit, ORDER_UP), 49)
            blk = [[[act[rb, nb][:RB // 2], act[rb, nb][RB // 2:]] for nb in range(4)]
                   for rb in range(4)]
            for p in range(7):
                for j, term in enumerate(lhs_terms2(blk, p)):
                    g[p * 7 + j].append(pack(*term))

        def down(n):
            left = [8, 8]

            def leaf(p):
                r = mm(as_bf16(jnp.concatenate(g[p], axis=1)),
                       as_bf16(w2_c[n, p].reshape(F // 8, LANE)))
                yield
                return [r]

            def emit(rb, nb, y):
                r = tile_rows(t, rb * RB, RB)
                xb[r, lanes(4 * n + nb)] = (hb[4 * n + nb, r, :] + y).astype(BF16)
                left[rb // 2] -= 1
                if not left[rb // 2]:
                    cp_y(t, n, rb // 2).start()
            yield from combine2(leaf, emit, ORDER_DOWN)

        side = ln2_sums(jnp.minimum(t + 1, NT - 1)) + ln2_stats(jnp.minimum(t + 2, NT - 1))
        run(chain(down(0), down(1)), 98, [pace.tick(w) for w in side], 0.05)
        pace.finish(sink.at[0], 1)
        return carry

    def prologue():
        early = [cp_q(k) for k in range(QPARTS)] + [cp_qkv(1), cp_qkv(2)]

        def start_early(k):
            for i, cp in enumerate(early):
                pl.when(k == i)(cp.start)
        cp_x(0).start()
        cp_x(1).start()

        def first_norm(t, carry):
            start_early(t)
            cp_x(t).wait()
            for stage in ln1(t, t):
                for w in stage:
                    w()
            return carry
        jax.lax.fori_loop(0, 2, first_norm, 0)

        def first_weights(g, carry):
            per_part = D // 32 // 4 // QPARTS

            @pl.when(g % per_part == 0)
            def _():
                start_early(2 + g // per_part)
                cp_q(g // per_part).wait()
            slabs = reorder_columns([qkv_slab(0, 4 * g + i, half)
                                     for i in range(4) for half in range(2)])
            for i in range(4):
                qkv_sums(0, 4 * g + i, slabs[2 * i], slabs[2 * i + 1])
            return carry
        jax.lax.fori_loop(0, D // 32 // 4, first_weights, 0)

        def first_projections(i, carry):
            pl.when(i == 0)(cp_wo().start)
            pl.when(i == 1)(cp_x(2).start)
            pl.when(i == 2)(cp_w1(0).start)
            pl.when(i > 0)(lambda: cp_qkv(jnp.maximum(i, 1)).wait())
            run(project(i & 1, i >> 1, qkv, 3 * (i & 1) + (i >> 1)), N_PROJ, prep_qkv(i), 0.0, 0.95)
            return carry
        jax.lax.fori_loop(0, 3, first_projections, 0)

        cp_w2(0).start()
        cp_wo().wait()
        work = prep_wo()
        pace = Pacer(3)
        run(project(0, 2, qkv, 2), N_PROJ, [pace.tick(w) for w in work])
        pace.finish(sink.at[1], 1)

        cp_x(3).start()
        cp_w1(NC - 1).start(priority=1)
        cp_w2(NC - 1).start(priority=1)
        cp_x(2).wait()
        first_halo()
        for j in range(NL):
            new[0, j, HALO:, :] = qkv[3, j, HALO:, :]
        pace = Pacer(7)
        stages = attention_work(pace, attention(qkv, True),
                                norm_riders(pace, ln1(2, 0), 0, 6, 16, 34))
        run(chain(project(1, 1, new, 1), project(1, 2, new, 2)), 2 * N_PROJ, sum(stages, []))
        pace.finish(sink.at[4], 0)
        cp_w1(NC - 1).wait()
        cp_w2(NC - 1).wait()

    def attention_step(t, carry):
        pl.when(t + 3 < NT)(lambda: cp_x(jnp.minimum(t + 3, NT - 1)).start())

        @pl.when(t < NC - 1)
        def _():
            cp_w1(t).start()
            cp_w2(t).start()
        cp_w1(t - 1).wait()
        cp_w2(t - 1).wait()
        pl.when(t + 2 < NT)(lambda: cp_x(jnp.minimum(t + 2, NT - 1)).wait())

        pace = Pacer(5)
        cut = 24
        moved_rows = [0, 0, 0]
        keys, values = hand_over(moved_rows)
        riders = [([pace.tick(w) for w in keys], 0, 7), ([pace.tick(w) for w in values], 0, 14),
                  ([pace.tick(w) for w in out_sums()], 0, 4)]
        riders += norm_riders(pace, ln1(jnp.minimum(t + 2, NT - 1), 0), 8, 16, cut, 34)
        riders.append(([w for p in prep_ffn(t - 1) for w in (pace.tick(p), pace.tick())], 0, 29))
        moved = [False] * 4

        def move_queries(n):
            for j in (n, n + 4):
                qkv[0, j, HALO:, :] = new[0, j, HALO:, :]
            moved[n] = True

        def check(m):
            def before(n):
                assert moved_rows[m] == TM
            return before
        stages = attention_work(pace, attention(qkv, moved=moved), riders)
        run(chain(project(0, 0, new, 0, move_queries), project(0, 1, new, 1, check(1)),
                  project(0, 2, new, 2, check(2))), 3 * N_PROJ, sum(stages[:cut], []))
        run(out_proj(t - 1, (0, 1), ORDER_PROJ), 2 * N_PROJ, sum(stages[cut:], []))
        pace.finish(sink.at[2], 1)
        return carry

    def epilogue():
        for m in (1, 2):
            for j in range(NL):
                new[m, j, 0:HALO, :] = qkv[m, j, TM:TM + HALO, :]
        for w in out_sums():
            w()
        pace = Pacer(11)
        norm = [pace.tick(w) for w in ln2_stats(0) + ln2_sums(0) + ln2_stats(1)]
        few = len(norm) // 5
        sums = out_sums()
        stages = attention_work(pace, attention(new),
                                [(norm[:few], 26, 34), (sums[:len(sums) // 2], 18, 19)], False)
        run(out_proj(NT - 2, (0, 1), ORDER_LAST), 2 * N_PROJ, sum(stages[:19], []))
        run(out_proj(NT - 1, (0,), ORDER_LAST), N_PROJ, sum(stages[19:], []) + sums[len(sums) // 2:])
        run(out_proj(NT - 1, (1,), ORDER_LAST), N_PROJ, norm[few:])
        pace.finish(sink.at[3], 0)

    prologue()
    jax.lax.fori_loop(1, NT - 1, attention_step, 0)
    epilogue()
    jax.lax.fori_loop(0, NT, ffn_step, 0)
    for t in range(NT):
        for k in range(4):
            cp_y(t, k // 2, k % 2).wait()


@jax.jit
def pallas_sequential_preLN__sliding_local_dilated__dense_activation_silu__prompt_kernel(
    A_x: jax.Array,
    A_wqkv: jax.Array,
    A_wo: jax.Array,
    B_x: jax.Array,
    B_w1: jax.Array,
    B_w2: jax.Array,
):
    del B_x
    vmem = pltpu.VMEM
    dma = pltpu.SemaphoreType.DMA
    hbm = pl.BlockSpec(memory_space=pl.ANY)
    out = pl.pallas_call(
        kernel,
        in_specs=[hbm] * 5,
        out_specs=hbm,
        out_shape=jax.ShapeDtypeStruct((S, D), BF16),
        scratch_shapes=[
            vmem((S, D), BF16),
            vmem((2, D // 2, 3 * D), BF16), vmem((D, D), BF16),
            vmem((NC, D, FC), BF16), vmem((NC, FC, D), BF16),
            vmem((3, 4 * 7, D // 4, LANE), U32),
            vmem((4 * 7, D // 4, LANE), U32),
            vmem((NC, 49, D // 8, LANE), U32),
            vmem((2, 49, NC, FC // 8, LANE), U32),
            vmem((2, 7, RA // 2, D // 2), U32),
            vmem((4, NL, TM + HALO, LANE), F32),
            vmem((3, NL, TM + HALO, LANE), F32),
            vmem((TM, D), F32), vmem((7 * TM // 2, D // 2), BF16),
            vmem((NL, S + 8, LANE), F32),
            vmem((2, S, LANE), F32), vmem((1, NL, TM, LANE), F32),
            vmem((1, 49, RB // 2, D // 4), U32),
            vmem((5, 8, LANE), F32), pltpu.SMEM((8,), I32),
            dma((NT,)), dma((3 + QPARTS,)), dma((NC,)), dma((NC,)), dma((4 * NT,)),
        ],
        compiler_params=pltpu.CompilerParams(vmem_limit_bytes=126 * 2 ** 20,
                                             disable_bounds_checks=True),
    )(A_x.reshape(S, D), A_wqkv.reshape(2, D // 2, 3 * D), A_wo, B_w1, B_w2)
    return out.reshape(1, S, D)
```

```python
import functools
import math
import operator

import jax
import jax.numpy as jnp
import jax.experimental.pallas as pl
import jax.experimental.pallas.tpu as pltpu

F32, BF16, U32, I32 = jnp.float32, jnp.bfloat16, jnp.uint32, jnp.int32

S, D, F = 2048, 1024, 3584
DH, WIN, DIL = 32, 8, 2
LANE = 128
NL = D // LANE
HALO = 16
EPS = 1e-5
LOG2E = math.log2(math.e)

TM = 256
NT = S // TM
RA = TM // 2
RO = TM // 4
RB = TM // 4
FC = 512
NC = F // FC
QPARTS = 4
SHARE = 3
N_PROJ = 4 * 7

ORDER_PROJ = (4, 2, 6, 0, 5, 3, 1)
ORDER_LAST = (5, 1, 3, 0, 2, 4, 6), (1, 3, 0, 5, 6, 4, 2), (6, 3, 1, 0, 2, 4, 5)
ORDER_UP = (6, 4, 2, 0, 3, 1, 5), (1, 3, 0, 6, 4, 2, 5)
ORDER_DOWN = (2, 4, 1, 3, 0, 5, 6), (2, 4, 1, 3, 0, 5, 6)


def _add(x, y):
    return [p + q for p, q in zip(x, y)]


def _sub(x, y):
    return [p - q for p, q in zip(x, y)]


def lhs_term(i, a11, a12, a21, a22):
    return (
        lambda: _add(a11, a22), lambda: _add(a21, a22), lambda: a11, lambda: a22,
        lambda: _add(a11, a12), lambda: _sub(a21, a11), lambda: _sub(a12, a22),
    )[i]()


def rhs_term(i, b11, b12, b21, b22):
    return (
        lambda: _add(b11, b22), lambda: b11, lambda: _sub(b12, b22), lambda: _sub(b21, b11),
        lambda: b22, lambda: _add(b11, b12), lambda: _add(b21, b22),
    )[i]()


RHS_BLOCKS = ((0, 3), (0,), (1, 3), (2, 0), (3,), (0, 1), (2, 3))
OUTPUTS = ({0: 1, 3: 1, 4: -1, 6: 1}, {2: 1, 4: 1}, {1: 1, 3: 1}, {0: 1, 1: -1, 2: 1, 5: 1})


def combine(product, emit, order):
    acc = [None] * 4
    left = [len(out) for out in OUTPUTS]
    for i in order:
        m = yield from product(i)
        for k, out in enumerate(OUTPUTS):
            if i in out:
                if acc[k] is None:
                    acc[k] = m, out[i]
                elif acc[k][1] < 0:
                    acc[k] = _sub(m, acc[k][0]), 1
                else:
                    acc[k] = (_add if out[i] > 0 else _sub)(acc[k][0], m), 1
                left[k] -= 1
                if not left[k]:
                    emit(k, acc[k][0])


def combine2(leaf, emit, orders):
    def outer(i):
        res = [None] * 4

        def keep(k, c):
            res[k] = c[0]
        yield from combine(lambda j: leaf(7 * i + j), keep, orders[1])
        return res

    def emit_outer(ko, cs):
        for ki in range(4):
            emit(2 * (ko // 2) + ki // 2, 2 * (ko % 2) + ki % 2, cs[ki])
    yield from combine(outer, emit_outer, orders[0])


def lhs_terms2(blk, i):
    outer = []
    for hi_r in range(2):
        for hi_c in range(2):
            flat = []
            for lo_r in range(2):
                for lo_c in range(2):
                    flat += blk[2 * hi_r + lo_r][2 * hi_c + lo_c]
            outer.append(flat)
    o = lhs_term(i, *outer)
    n = len(o) // 4
    inner = [o[q * n:(q + 1) * n] for q in range(4)]
    return [lhs_term(j, *inner) for j in range(7)]


def pack(lo, hi):
    return pltpu.bitcast(pltpu.pack_elementwise([lo, hi], packed_dtype=BF16), U32)


def unpack(w):
    return [pltpu.unpack_elementwise(w, index=i, packed_dtype=BF16, unpacked_dtype=F32)
            for i in range(2)]


def as_bf16(w):
    return pltpu.bitcast(w, BF16)


def mm(a, b):
    return jnp.dot(a, b, preferred_element_type=F32)


def total(xs):
    return functools.reduce(operator.add, xs)


def lane_mean(part):
    return jnp.sum(part, axis=1, keepdims=True) * (1.0 / D)


def aligned(start, size):
    return pl.ds(start if isinstance(start, int) else pl.multiple_of(start, size), size)


def lanes(j, n=1):
    return slice(j * LANE, (j + n) * LANE)


def chain(*gens):
    for g in gens:
        yield from g


def run(main, n_main, side=()):
    done = step = 0
    for _ in main:
        step += 1
        want = min(len(side), math.ceil(step / n_main * len(side)))
        while done < want:
            side[done]()
            done += 1
    assert step == n_main and done == len(side)


class Pacer:
    def __init__(self, width):
        self.state = [jnp.full((8, LANE), k, U32) for k in range(width)]
        self.count = 0

    def tick(self, piece=None):
        def thunk():
            k = self.count % len(self.state)
            self.count += 1
            v = self.state[k]
            if piece is not None:
                v = v ^ pltpu.bitcast(piece(), U32)
            self.state[k] = pltpu.roll(v, 1, 1)
        return thunk

    def finish(self, sink, tail):
        out = []
        for j in range(len(self.state)):
            x = pltpu.bitcast(self.state[(self.count - 1 - j) % len(self.state)], F32)
            for _ in range(j * tail):
                x = jnp.tanh(x)
            out.append(x)
        sink[...] = total(out)


def kernel(x_hbm, wqkv_hbm, wo_hbm, w1_hbm, w2_hbm, out_hbm,
           xb, wqkv_raw, wo_raw, w1_raw, w2_raw,
           wqkv_c, wo_c, w1_c, w2_c,
           a1, qkv, new, ob, o_c,
           hb, stats, zb, a2, sink, zero, sem_x, sem_w, sem_1, sem_2, sem_y):
    for k in range(8):
        zero[k] = 0

    def tile_rows(t, off, n, stride=1):
        base = t * TM if isinstance(t, int) else pl.multiple_of(t * TM, TM)
        return pl.ds(base + off, n, stride=stride)

    def cp_x(t):
        rows = tile_rows(t, 0, TM)
        return pltpu.make_async_copy(x_hbm.at[rows], xb.at[rows], sem_x.at[t])

    def cp_qkv(m):
        src, dst = (r.at[:, :, aligned(m * D, D)] for r in (wqkv_hbm, wqkv_raw))
        return pltpu.make_async_copy(src, dst, sem_w.at[m])

    def cp_q(part):
        n = D // 2 // QPARTS
        src, dst = (r.at[:, aligned(part * n, n), pl.ds(0, D)] for r in (wqkv_hbm, wqkv_raw))
        return pltpu.make_async_copy(src, dst, sem_w.at[3 + part])

    def cp_wo():
        return pltpu.make_async_copy(wo_hbm, wo_raw, sem_w.at[0])

    def cp_w1(c):
        return pltpu.make_async_copy(w1_hbm.at[:, aligned(c * FC, FC)], w1_raw.at[c], sem_1.at[c])

    def cp_w2(c):
        return pltpu.make_async_copy(w2_hbm.at[aligned(c * FC, FC)], w2_raw.at[c], sem_2.at[c])

    def cp_y(t, n, rh):
        src, dst = (r.at[tile_rows(t, rh * TM // 2, TM // 2), pl.ds(n * D // 2, D // 2)]
                    for r in (xb, out_hbm))
        return pltpu.make_async_copy(src, dst, sem_y.at[4 * t + 2 * n + rh])

    def reorder_columns(groups):
        l = jax.lax.broadcasted_iota(I32, (8, LANE), 1)
        groups = [[g[-t % NL] for t in range(NL)] for g in groups]
        for b in (1, 2, 4):
            move = (l & b) != 0
            groups = [[jnp.where(move, g[(t - b) % NL], g[t]) for t in range(NL)] for g in groups]
        e = l >> 5
        a = (l >> 1) & 3
        j = ((l >> 3) & 1) | ((l & 1) << 1) | (((l >> 4) & 1) << 2)
        out = [[None] * NL for _ in groups]
        for t in range(NL):
            for k, g in enumerate(groups):
                out[k][t] = jnp.take_along_axis(g[t], 32 * a + 8 * e + ((j + t) & 7), axis=1)
        return out

    def qkv_slab(m, i, half):
        w = pltpu.bitcast(wqkv_raw[half, aligned(16 * i, 16), aligned(m * D, D)], U32)
        return [w[:, lanes(j)] for j in range(NL)]

    def qkv_sums(m, i, top, bottom):
        for t in range(4):
            raw = (top[t], top[t + 4], bottom[t], bottom[t + 4])
            blk = [unpack(w) for w in raw]
            for p in range(7):
                w = raw[0] if p == 1 else raw[3] if p == 4 else pack(*rhs_term(p, *blk))
                wqkv_c[m, t * 7 + p, aligned(8 * i, 8), :] = w

    def prep_qkv(m):
        held = {}

        def reorder(i, half):
            held[half], = reorder_columns([qkv_slab(m, i, half)])
        return [w for i in range(D // 32) for w in (
            functools.partial(reorder, i, 0), functools.partial(reorder, i, 1),
            lambda i=i: qkv_sums(m, i, held[0], held[1]))]

    def prep_wo():
        def staged(e, j, a):
            return 9 * (32 * e + 8 * (j >> 1) + 4 * (j & 1) + a)

        def widen(i):
            j, a = i // 4, i % 4
            seen = []
            for n in range(NL):
                w = wo_raw[32 * i:32 * (i + 1), lanes(n)].astype(F32)
                for e in range(4):
                    g = w[8 * e:8 * e + 8]
                    hb[n, pl.ds(staged(e, j, a), 8), :] = pltpu.roll(g, 8 - j, 0) if j else g
                seen.append(g)
            return total(seen)

        def rows(n, t, e, j_hi):
            return [hb[n, pl.ds(staged(e, 4 * j_hi + 2 * j_mid, 0) + t, 8, stride=9), :]
                    for j_mid in range(2)]

        def sums(n, t, e):
            seen = []
            for j_hi in range(2):
                blk = [rows(n, t, e, j_hi), rows(n + 4, t, e, j_hi),
                       rows(n, t + 4, e, j_hi), rows(n + 4, t + 4, e, j_hi)]
                r = 64 * t + 16 * e + 8 * j_hi
                words = [pack(*rhs_term(p, *blk)) for p in range(7)]
                for p in range(7):
                    wo_c[n * 7 + p, r:r + 8, :] = words[p]
                seen.append(words[5] ^ words[6])
            return seen[0] ^ seen[1]

        return ([functools.partial(widen, i) for i in range(D // 32)]
                + [functools.partial(sums, n, t, e)
                   for n in range(4) for t in range(4) for e in range(4)])

    def prep_ffn(step):
        groups = ((1, 5), (2, 4, 0), (3, 6))

        def piece(load, store, group):
            held = {}

            def block(q):
                if q not in held:
                    held[q] = [x for r in range(2) for c in range(2)
                               for x in unpack(load(2 * (q // 2) + r, 2 * (q % 2) + c))]
                return held[q]
            for p in group:
                o = rhs_term(p, *[block(q) if q in RHS_BLOCKS[p] else None for q in range(4)])
                words = [pack(*rhs_term(j, o[0:2], o[2:4], o[4:6], o[6:8])) for j in range(7)]
                for j in range(7):
                    store(p * 7 + j, words[j])
            return words[2] ^ words[3]

        def up(c, i, n):
            def load(r, b):
                rows = aligned(256 * r + 16 * i, 16)
                return pltpu.bitcast(w1_raw[c + zero[n], rows, lanes(b)], U32)

            def store(p, word):
                w1_c[c, p, aligned(8 * i, 8), :] = word
            return piece(load, store, groups[n])

        def down(c, g, n):
            i, half = g >> 1, g & 1

            def load(r, b):
                return pltpu.bitcast(w2_raw[c + zero[n], aligned(128 * r + 16 * i, 16),
                                            aligned((4 * half + b) * LANE, LANE)], U32)

            def store(p, word):
                w2_c[half, p, c, aligned(8 * i, 8), :] = word
            return piece(load, store, groups[n])

        slabs = [(NC - 1, jnp.minimum(SHARE * step + i, 15)) for i in range(SHARE)]
        slabs += [(step, i) for i in range(16)]
        return [functools.partial(f, c, i, n) for c, i in slabs for f in (up, down)
                for n in range(len(groups))]

    def ln1(t, slot):
        mean, inv = {}, {}

        def load(k, rh, i, cols):
            return pltpu.bitcast(xb[tile_rows(t + zero[k], rh * RA + 16 * i, 16), cols], U32)

        def rows_of(k, rh, i):
            w = load(k, rh, i, slice(None))
            return zip(*[unpack(w[:, lanes(j)]) for j in range(NL)])

        def means(rh, i):
            part = [total(x) for x in rows_of(0, rh, i)]
            mean[rh, i] = [lane_mean(p) for p in part]
            return total(part)

        def scales(rh, i):
            part = [total([(u - m) * (u - m) for u in x])
                    for x, m in zip(rows_of(1, rh, i), mean[rh, i])]
            inv[rh, i] = [jax.lax.rsqrt(lane_mean(p) + EPS) for p in part]
            return total(part)

        def sums(i, j):
            blk = [[(u - m) * r for u, m, r in zip(unpack(load(2, rh, i, lanes(j + 4 * kh))),
                                                   mean[rh, i], inv[rh, i])]
                   for rh in range(2) for kh in range(2)]
            words = [pack(*lhs_term(p, *blk)) for p in range(7)]
            for p in range(7):
                a1[slot, p, 8 * i:8 * i + 8, lanes(j)] = words[p]
            return words[5] ^ words[6]

        groups = [(rh, i) for i in range(RA // 16) for rh in range(2)]
        return ([functools.partial(means, *g) for g in groups],
                [functools.partial(scales, *g) for g in groups],
                [functools.partial(sums, i, j) for i in range(RA // 16) for j in range(4)])

    def project(slot, m, buf, dst, before=None):
        for n in range(4):
            if before:
                before(n)

            def product(p):
                r = mm(as_bf16(a1[slot, p]), as_bf16(wqkv_c[m, n * 7 + p]))
                yield
                return [r]

            def emit(k, c):
                r = HALO + (k // 2) * RA
                buf[dst, n + 4 * (k % 2), r:r + RA, :] = c[0]
            yield from combine(product, emit, ORDER_PROJ)

    def first_halo():
        for j in range(NL):
            qkv[1, j, 0:HALO, :] = jnp.zeros((HALO, LANE), F32)
            qkv[2, j, 0:HALO, :] = jnp.broadcast_to(qkv[2, j, HALO:HALO + 1, :], (HALO, LANE))

    def hand_over(moved_rows):
        def move(m, r, n):
            for j in range(NL):
                qkv[m, j, HALO + r:HALO + r + n, :] = new[m, j, HALO + r:HALO + r + n, :]
            moved_rows[m] += n
            return qkv[m + zero[7], 0, HALO + r:HALO + r + 8, :]
        for m in (1, 2):
            for j in range(NL):
                qkv[m, j, 0:HALO, :] = qkv[m, j, TM:TM + HALO, :]
            move(m, 0, 16)
        return [[functools.partial(move, m, r, 24) for r in range(16, TM, 24)] for m in (1, 2)]

    def attention(buf, first=False, moved=(True,) * 4):
        held = {}

        def window(r, w):
            return pl.ds(HALO + r - DIL * w, 8)

        def score(r, w):
            if w == 0:
                held[r, "q"] = [(buf if moved[j % 4] else new)[0, j, HALO + r:HALO + r + 8, :]
                                for j in range(NL)]
            a = total([held[r, "q"][j] * buf[1, j, window(r, w), :] for j in range(NL)])
            held[r, w] = a + pltpu.roll(a, 64, 1)

        def logit(r, w):
            a = (held[r, w] + pltpu.roll(held[r, w], 32, 1)) * (DH ** -0.5 * LOG2E)
            if first and r < DIL * w:
                pos = r + jax.lax.broadcasted_iota(I32, (8, LANE), 0)
                a = jnp.where(pos >= DIL * w, a, -1e9 * LOG2E)
            held[r, w] = a
            held[r, "max"] = a if w == 0 else jnp.maximum(held[r, "max"], a)

        def softmax(r):
            ex = [jnp.exp2(held[r, w] - held[r, "max"]) for w in range(WIN)]
            inv = 1.0 / total(ex)
            held[r] = [e * inv for e in ex]

        def value(r, j):
            o = total([held[r][w] * buf[2, j, window(r, w), :] for w in range(WIN)])
            ob[r:r + 8, lanes(j)] = o
            return o

        return [([functools.partial(score, r, w) for w in range(WIN)],
                 [functools.partial(logit, r, w) for w in range(WIN)],
                 functools.partial(softmax, r),
                 [functools.partial(value, r, j) for j in range(NL)]) for r in range(0, TM, 8)]

    def attention_work(pace, att, riders, pattern, lead=True):
        stages = []
        n = len(att)
        placed = [0] * len(riders)
        for u in range(n + 2):
            work = []
            stages.append(work)
            for w in range(WIN):
                k = 0
                for what in pattern:
                    if what == "s" and u < n:
                        work.append(att[u][0][w])
                    if what == "l" and 1 <= u <= n:
                        work.append(att[u - 1][1][w])
                    if what == "v" and (u >= 2 or lead):
                        work.append(pace.tick(att[u - 2][3][w] if u >= 2 else None))
                    if what == "r":
                        thunks, lo, hi = riders[k]
                        want = (WIN * (u - lo) + w + 1) * len(thunks) // (WIN * (hi - lo))
                        want = min(len(thunks), max(0, want))
                        work += thunks[placed[k]:want]
                        placed[k] = want
                        k += 1
            if 1 <= u <= n:
                work.append(att[u - 1][2])
        assert placed == [len(thunks) for thunks, _, _ in riders]
        return stages

    def norm_riders(pace, norm, *bounds):
        return [([pace.tick(w) for w in stage], lo, hi)
                for stage, lo, hi in zip(norm, bounds, bounds[1:])]

    def out_sums():
        def unit(s, i):
            blk = []
            for rh in range(2):
                r = (2 * s + rh) * RO + 16 * i
                blk += [[ob[r:r + 16, lanes(4 * kh, 4)]] for kh in range(2)]
            terms = [lhs_term(p, *blk)[0] for p in range(7)]
            for p in range(7):
                r = (s * 7 + p) * RO + 16 * i
                o_c[r:r + 16, :] = terms[p].astype(BF16)
            return terms[5][0:8, lanes(0)] + terms[6][8:16, lanes(3)]
        return [functools.partial(unit, s, i) for s in range(2) for i in range(RO // 16)]

    def out_proj(t, halves, order):
        for s in halves:
            for n in range(4):
                def product(p):
                    r = mm(o_c[(s * 7 + p) * RO:(s * 7 + p + 1) * RO, :], as_bf16(wo_c[n * 7 + p]))
                    yield
                    return [r]

                def emit(k, c):
                    r = tile_rows(t, (2 * s + k // 2) * RO, RO)
                    j = n + 4 * (k % 2)
                    hb[j, r, :] = xb[r, lanes(j)].astype(F32) + c[0]
                yield from combine(product, emit, order)

    def quad_rows(t, rb, i):
        return tile_rows(t, rb * RB + 32 * (i % 2) + i // 2, 8, stride=4)

    def ln2_stats(t):
        def means(rb, i):
            part = total([hb[j, quad_rows(t, rb, i), :] for j in range(NL)])
            stats[0, tile_rows(t, rb * RB + 8 * i, 8), :] = jnp.broadcast_to(lane_mean(part), (8, LANE))
            return part

        def scales(rb, i):
            dst = tile_rows(t, rb * RB + 8 * i, 8)
            mean = stats[0, dst, :]
            cen = [hb[j, quad_rows(t + zero[6], rb, i), :] - mean for j in range(NL)]
            part = total([u * u for u in cen])
            stats[1, dst, :] = jnp.broadcast_to(0.5 * jax.lax.rsqrt(lane_mean(part) + EPS), (8, LANE))
            return part
        return [functools.partial(f, rb, i) for f in (means, scales) for rb in range(4) for i in range(8)]

    def ln2_sums(t):
        z = zero[1]

        def norm(rb, i):
            src = tile_rows(t, rb * RB + 8 * i, 8)
            mean, inv = stats[0, src, :], stats[1, src, :]
            r = rb * RB + 8 * i
            out = [(hb[j, quad_rows(t, rb, i), :] - mean) * inv for j in range(NL)]
            for j in range(NL):
                zb[z, j, r:r + 8, :] = out[j]
            return total(out)

        def sums(i, n, p):
            blk = [[[zb[zero[2 + p % 4], 2 * c + n, pl.ds(rb * RB + 8 * (i + 4 * h), 8), :]
                     for h in range(2)] for c in range(4)] for rb in range(4)]
            words = [pack(*term) for term in lhs_terms2(blk, p)]
            for j in range(7):
                a2[0, p * 7 + j, 8 * i:8 * i + 8, lanes(n)] = words[j]
            return words[5] ^ words[6]

        return ([functools.partial(norm, rb, i + 4 * h)
                 for i in range(4) for rb in range(4) for h in range(2)]
                + [functools.partial(sums, i, n, p)
                   for i in range(4) for n in range(2) for p in range(7)])

    def ffn_step(t, carry):
        g = [[] for _ in range(49)]
        pace = Pacer(1)
        for c in range(NC):
            act = {}

            def leaf(p):
                r = mm(as_bf16(a2[0, p]), as_bf16(w1_c[c, p]))
                yield
                return [r]

            def emit(rb, nb, v):
                act[rb, nb] = v * jnp.tanh(v) + v
            run(combine2(leaf, emit, ORDER_UP), 49)
            blk = [[[act[rb, nb][:RB // 2], act[rb, nb][RB // 2:]] for nb in range(4)]
                   for rb in range(4)]
            for p in range(7):
                for j, term in enumerate(lhs_terms2(blk, p)):
                    g[p * 7 + j].append(pack(*term))

        def down(n):
            left = [8, 8]

            def leaf(p):
                r = mm(as_bf16(jnp.concatenate(g[p], axis=1)),
                       as_bf16(w2_c[n, p].reshape(F // 8, LANE)))
                yield
                return [r]

            def emit(rb, nb, y):
                r = tile_rows(t, rb * RB, RB)
                xb[r, lanes(4 * n + nb)] = (hb[4 * n + nb, r, :] + y).astype(BF16)
                left[rb // 2] -= 1
                if not left[rb // 2]:
                    cp_y(t, n, rb // 2).start()
            yield from combine2(leaf, emit, ORDER_DOWN)

        sums = ln2_sums(jnp.minimum(t + 1, NT - 1))
        moments = ln2_stats(jnp.minimum(t + 2, NT - 1))
        side = sums[:32] + moments[:32] + sums[32:46] + moments[32:] + sums[46:]
        run(chain(down(0), down(1)), 98, [pace.tick(w) for w in side])
        pace.finish(sink.at[0], 1)
        return carry

    def prologue():
        early = [cp_q(k) for k in range(QPARTS)] + [cp_qkv(1), cp_qkv(2)]

        def start_early(k):
            for i, cp in enumerate(early):
                pl.when(k == i)(cp.start)
        cp_x(0).start()
        cp_x(1).start()

        def first_norm(t, carry):
            start_early(t)
            cp_x(t).wait()
            for stage in ln1(t, t):
                for w in stage:
                    w()
            return carry
        jax.lax.fori_loop(0, 2, first_norm, 0)

        def first_weights(g, carry):
            per_part = D // 32 // 4 // QPARTS

            @pl.when(g % per_part == 0)
            def _():
                start_early(2 + g // per_part)
                cp_q(g // per_part).wait()
            slabs = reorder_columns([qkv_slab(0, 4 * g + i, half)
                                     for i in range(4) for half in range(2)])
            for i in range(4):
                qkv_sums(0, 4 * g + i, slabs[2 * i], slabs[2 * i + 1])
            return carry
        jax.lax.fori_loop(0, D // 32 // 4, first_weights, 0)

        def first_projections(i, carry):
            pl.when(i == 0)(cp_wo().start)
            pl.when(i == 1)(cp_x(2).start)
            pl.when(i == 2)(cp_w1(0).start)
            pl.when(i > 0)(lambda: cp_qkv(jnp.maximum(i, 1)).wait())
            run(project(i & 1, i >> 1, qkv, 3 * (i & 1) + (i >> 1)), N_PROJ, prep_qkv(i))
            return carry
        jax.lax.fori_loop(0, 3, first_projections, 0)

        cp_w2(0).start()
        cp_wo().wait()
        work = prep_wo()
        pace = Pacer(3)
        run(project(0, 2, qkv, 2), N_PROJ, [pace.tick(w) for w in work])
        pace.finish(sink.at[1], 1)

        cp_x(3).start()
        cp_w1(NC - 1).start(priority=1)
        cp_w2(NC - 1).start(priority=1)
        cp_x(2).wait()
        first_halo()
        for j in range(NL):
            new[0, j, HALO:, :] = qkv[3, j, HALO:, :]
        pace = Pacer(7)
        norm = norm_riders(pace, ln1(2, 0), 0, 6, 16, 34)
        stages = attention_work(pace, attention(qkv, True), [norm[1], norm[0], norm[2]], "svlrrr")
        run(chain(project(1, 1, new, 1), project(1, 2, new, 2)), 2 * N_PROJ, sum(stages, []))
        pace.finish(sink.at[4], 0)
        cp_w1(NC - 1).wait()
        cp_w2(NC - 1).wait()

    def attention_step(t, carry):
        pl.when(t + 3 < NT)(lambda: cp_x(jnp.minimum(t + 3, NT - 1)).start())

        @pl.when(t < NC - 1)
        def _():
            cp_w1(t).start()
            cp_w2(t).start()
        cp_w1(t - 1).wait()
        cp_w2(t - 1).wait()
        pl.when(t + 2 < NT)(lambda: cp_x(jnp.minimum(t + 2, NT - 1)).wait())

        pace = Pacer(5)
        cut = 24
        moved_rows = [0, 0, 0]
        keys, values = hand_over(moved_rows)
        norm = norm_riders(pace, ln1(jnp.minimum(t + 2, NT - 1), 0), 8, 16, cut, 34)
        riders = [([pace.tick(w) for w in keys], 0, 7),
                  norm[1],
                  ([w for p in prep_ffn(t - 1) for w in (pace.tick(p), pace.tick())], 0, 29),
                  norm[0],
                  norm[2],
                  ([pace.tick(w) for w in values], 0, 14),
                  ([pace.tick(w) for w in out_sums()], 0, 4)]
        moved = [False] * 4

        def move_queries(n):
            for j in (n, n + 4):
                qkv[0, j, HALO:, :] = new[0, j, HALO:, :]
            moved[n] = True

        def check(m):
            def before(n):
                assert moved_rows[m] == TM
            return before
        stages = attention_work(pace, attention(qkv, moved=moved), riders, "slvrrrrrrr")
        run(chain(project(0, 0, new, 0, move_queries), project(0, 1, new, 1, check(1)),
                  project(0, 2, new, 2, check(2))), 3 * N_PROJ, sum(stages[:cut], []))
        run(out_proj(t - 1, (0, 1), ORDER_PROJ), 2 * N_PROJ, sum(stages[cut:], []))
        pace.finish(sink.at[2], 1)
        return carry

    def epilogue():
        for m in (1, 2):
            for j in range(NL):
                new[m, j, 0:HALO, :] = qkv[m, j, TM:TM + HALO, :]
        for w in out_sums():
            w()
        pace = Pacer(11)
        norm = [pace.tick(w) for w in ln2_stats(0) + ln2_sums(0) + ln2_stats(1)]
        few = len(norm) // 5
        sums = out_sums()
        stages = attention_work(pace, attention(new),
                                [(norm[:few], 26, 34), (sums[:len(sums) // 2], 18, 19)],
                                "lrvsr", False)
        run(out_proj(NT - 2, (0, 1), ORDER_LAST[0]), 2 * N_PROJ, sum(stages[:19], []))
        run(out_proj(NT - 1, (0,), ORDER_LAST[1]), N_PROJ,
            sum(stages[19:], []) + sums[len(sums) // 2:])
        run(out_proj(NT - 1, (1,), ORDER_LAST[2]), N_PROJ, norm[few:])
        pace.finish(sink.at[3], 0)

    prologue()
    jax.lax.fori_loop(1, NT - 1, attention_step, 0)
    epilogue()
    jax.lax.fori_loop(0, NT, ffn_step, 0)
    for t in range(NT):
        for k in range(4):
            cp_y(t, k // 2, k % 2).wait()


@jax.jit
def pallas_sequential_preLN__sliding_local_dilated__dense_activation_silu__prompt_kernel(
    A_x: jax.Array,
    A_wqkv: jax.Array,
    A_wo: jax.Array,
    B_x: jax.Array,
    B_w1: jax.Array,
    B_w2: jax.Array,
):
    del B_x
    vmem = pltpu.VMEM
    dma = pltpu.SemaphoreType.DMA
    hbm = pl.BlockSpec(memory_space=pl.ANY)
    out = pl.pallas_call(
        kernel,
        in_specs=[hbm] * 5,
        out_specs=hbm,
        out_shape=jax.ShapeDtypeStruct((S, D), BF16),
        scratch_shapes=[
            vmem((S, D), BF16),
            vmem((2, D // 2, 3 * D), BF16), vmem((D, D), BF16),
            vmem((NC, D, FC), BF16), vmem((NC, FC, D), BF16),
            vmem((3, 4 * 7, D // 4, LANE), U32),
            vmem((4 * 7, D // 4, LANE), U32),
            vmem((NC, 49, D // 8, LANE), U32),
            vmem((2, 49, NC, FC // 8, LANE), U32),
            vmem((2, 7, RA // 2, D // 2), U32),
            vmem((4, NL, TM + HALO, LANE), F32),
            vmem((3, NL, TM + HALO, LANE), F32),
            vmem((TM, D), F32), vmem((7 * TM // 2, D // 2), BF16),
            vmem((NL, S + 8, LANE), F32),
            vmem((2, S, LANE), F32), vmem((1, NL, TM, LANE), F32),
            vmem((1, 49, RB // 2, D // 4), U32),
            vmem((5, 8, LANE), F32), pltpu.SMEM((8,), I32),
            dma((NT,)), dma((3 + QPARTS,)), dma((NC,)), dma((NC,)), dma((4 * NT,)),
        ],
        compiler_params=pltpu.CompilerParams(vmem_limit_bytes=126 * 2 ** 20,
                                             disable_bounds_checks=True),
    )(A_x.reshape(S, D), A_wqkv.reshape(2, D // 2, 3 * D), A_wo, B_w1, B_w2)
    return out.reshape(1, S, D)
```

```python
import functools
import math
import operator

import jax
import jax.numpy as jnp
import jax.experimental.pallas as pl
import jax.experimental.pallas.tpu as pltpu

F32, BF16, U32, I32 = jnp.float32, jnp.bfloat16, jnp.uint32, jnp.int32

S, D, F = 2048, 1024, 3584
DH, WIN, DIL = 32, 8, 2
LANE = 128
NL = D // LANE
HALO = 16
EPS = 1e-5
LOG2E = math.log2(math.e)

TM = 256
NT = S // TM
RA = TM // 2
RO = TM // 4
RB = TM // 4
FC = 512
NC = F // FC
QPARTS = 4
SHARE = 3
N_PROJ = 4 * 7

ORDER_PROJ = (4, 2, 6, 0, 5, 3, 1)
ORDER_FIRST_V = (4, 6, 2, 0, 3, 5, 1)
ORDER_STEP = (3, 1, 0, 6, 4, 2, 5), (4, 2, 6, 0, 5, 3, 1), (4, 2, 0, 6, 5, 3, 1)
ORDER_LAST = (5, 1, 3, 0, 2, 4, 6), (1, 3, 0, 5, 6, 4, 2), (6, 3, 1, 0, 2, 4, 5)
ORDER_UP = (6, 4, 2, 0, 3, 1, 5), (1, 3, 0, 6, 4, 2, 5)
ORDER_DOWN = (2, 4, 1, 3, 0, 5, 6), (2, 4, 1, 3, 0, 5, 6)


def _add(x, y):
    return [p + q for p, q in zip(x, y)]


def _sub(x, y):
    return [p - q for p, q in zip(x, y)]


def lhs_term(i, a11, a12, a21, a22):
    return (
        lambda: _add(a11, a22), lambda: _add(a21, a22), lambda: a11, lambda: a22,
        lambda: _add(a11, a12), lambda: _sub(a21, a11), lambda: _sub(a12, a22),
    )[i]()


def rhs_term(i, b11, b12, b21, b22):
    return (
        lambda: _add(b11, b22), lambda: b11, lambda: _sub(b12, b22), lambda: _sub(b21, b11),
        lambda: b22, lambda: _add(b11, b12), lambda: _add(b21, b22),
    )[i]()


RHS_BLOCKS = ((0, 3), (0,), (1, 3), (2, 0), (3,), (0, 1), (2, 3))
OUTPUTS = ({0: 1, 3: 1, 4: -1, 6: 1}, {2: 1, 4: 1}, {1: 1, 3: 1}, {0: 1, 1: -1, 2: 1, 5: 1})


def combine(product, emit, order):
    acc = [None] * 4
    left = [len(out) for out in OUTPUTS]
    for i in order:
        m = yield from product(i)
        for k, out in enumerate(OUTPUTS):
            if i in out:
                if acc[k] is None:
                    acc[k] = m, out[i]
                elif acc[k][1] < 0:
                    acc[k] = _sub(m, acc[k][0]), 1
                else:
                    acc[k] = (_add if out[i] > 0 else _sub)(acc[k][0], m), 1
                left[k] -= 1
                if not left[k]:
                    emit(k, acc[k][0])


def combine2(leaf, emit, orders):
    def outer(i):
        res = [None] * 4

        def keep(k, c):
            res[k] = c[0]
        yield from combine(lambda j: leaf(7 * i + j), keep, orders[1])
        return res

    def emit_outer(ko, cs):
        for ki in range(4):
            emit(2 * (ko // 2) + ki // 2, 2 * (ko % 2) + ki % 2, cs[ki])
    yield from combine(outer, emit_outer, orders[0])


def lhs_terms2(blk, i):
    outer = []
    for hi_r in range(2):
        for hi_c in range(2):
            flat = []
            for lo_r in range(2):
                for lo_c in range(2):
                    flat += blk[2 * hi_r + lo_r][2 * hi_c + lo_c]
            outer.append(flat)
    o = lhs_term(i, *outer)
    n = len(o) // 4
    inner = [o[q * n:(q + 1) * n] for q in range(4)]
    return [lhs_term(j, *inner) for j in range(7)]


def pack(lo, hi):
    return pltpu.bitcast(pltpu.pack_elementwise([lo, hi], packed_dtype=BF16), U32)


def unpack(w):
    return [pltpu.unpack_elementwise(w, index=i, packed_dtype=BF16, unpacked_dtype=F32)
            for i in range(2)]


def as_bf16(w):
    return pltpu.bitcast(w, BF16)


def mm(a, b):
    return jnp.dot(a, b, preferred_element_type=F32)


def total(xs):
    return functools.reduce(operator.add, xs)


def lane_mean(part):
    return jnp.sum(part, axis=1, keepdims=True) * (1.0 / D)


def aligned(start, size):
    return pl.ds(start if isinstance(start, int) else pl.multiple_of(start, size), size)


def lanes(j, n=1):
    return slice(j * LANE, (j + n) * LANE)


def chain(*gens):
    for g in gens:
        yield from g


def run(main, n_main, side=()):
    done = step = 0
    for _ in main:
        step += 1
        want = min(len(side), math.ceil(step / n_main * len(side)))
        while done < want:
            side[done]()
            done += 1
    assert step == n_main and done == len(side)


class Pacer:
    def __init__(self, width):
        self.state = [jnp.full((8, LANE), k, U32) for k in range(width)]
        self.count = 0

    def tick(self, piece=None):
        def thunk():
            k = self.count % len(self.state)
            self.count += 1
            v = self.state[k]
            if piece is not None:
                v = v ^ pltpu.bitcast(piece(), U32)
            self.state[k] = pltpu.roll(v, 1, 1)
        return thunk

    def finish(self, sink, tail):
        out = []
        for j in range(len(self.state)):
            x = pltpu.bitcast(self.state[(self.count - 1 - j) % len(self.state)], F32)
            for _ in range(j * tail):
                x = jnp.tanh(x)
            out.append(x)
        sink[...] = total(out)


def kernel(x_hbm, wqkv_hbm, wo_hbm, w1_hbm, w2_hbm, out_hbm,
           xb, wqkv_raw, wo_raw, w1_raw, w2_raw,
           wqkv_c, wo_c, w1_c, w2_c,
           a1, qkv, new, ob, o_c,
           hb, stats, zb, a2, sink, zero, sem_x, sem_w, sem_1, sem_2, sem_y):
    for k in range(8):
        zero[k] = 0

    def tile_rows(t, off, n, stride=1):
        base = t * TM if isinstance(t, int) else pl.multiple_of(t * TM, TM)
        return pl.ds(base + off, n, stride=stride)

    def cp_x(t):
        rows = tile_rows(t, 0, TM)
        return pltpu.make_async_copy(x_hbm.at[rows], xb.at[rows], sem_x.at[t])

    def cp_qkv(m):
        src, dst = (r.at[:, :, aligned(m * D, D)] for r in (wqkv_hbm, wqkv_raw))
        return pltpu.make_async_copy(src, dst, sem_w.at[m])

    def cp_q(part):
        n = D // 2 // QPARTS
        src, dst = (r.at[:, aligned(part * n, n), pl.ds(0, D)] for r in (wqkv_hbm, wqkv_raw))
        return pltpu.make_async_copy(src, dst, sem_w.at[3 + part])

    def cp_wo():
        return pltpu.make_async_copy(wo_hbm, wo_raw, sem_w.at[0])

    def cp_w1(c):
        return pltpu.make_async_copy(w1_hbm.at[:, aligned(c * FC, FC)], w1_raw.at[c], sem_1.at[c])

    def cp_w2(c):
        return pltpu.make_async_copy(w2_hbm.at[aligned(c * FC, FC)], w2_raw.at[c], sem_2.at[c])

    def cp_y(t, n, rh):
        src, dst = (r.at[tile_rows(t, rh * TM // 2, TM // 2), pl.ds(n * D // 2, D // 2)]
                    for r in (xb, out_hbm))
        return pltpu.make_async_copy(src, dst, sem_y.at[4 * t + 2 * n + rh])

    def reorder_columns(groups):
        l = jax.lax.broadcasted_iota(I32, (8, LANE), 1)
        groups = [[g[-t % NL] for t in range(NL)] for g in groups]
        for b in (1, 2, 4):
            move = (l & b) != 0
            groups = [[jnp.where(move, g[(t - b) % NL], g[t]) for t in range(NL)] for g in groups]
        e = l >> 5
        a = (l >> 1) & 3
        j = ((l >> 3) & 1) | ((l & 1) << 1) | (((l >> 4) & 1) << 2)
        out = [[None] * NL for _ in groups]
        for t in range(NL):
            for k, g in enumerate(groups):
                out[k][t] = jnp.take_along_axis(g[t], 32 * a + 8 * e + ((j + t) & 7), axis=1)
        return out

    def qkv_slab(m, i, half):
        w = pltpu.bitcast(wqkv_raw[half, aligned(16 * i, 16), aligned(m * D, D)], U32)
        return [w[:, lanes(j)] for j in range(NL)]

    def qkv_sums(m, i, top, bottom):
        for t in range(4):
            raw = (top[t], top[t + 4], bottom[t], bottom[t + 4])
            blk = [unpack(w) for w in raw]
            for p in range(7):
                w = raw[0] if p == 1 else raw[3] if p == 4 else pack(*rhs_term(p, *blk))
                wqkv_c[m, t * 7 + p, aligned(8 * i, 8), :] = w

    def prep_qkv(m):
        held = {}

        def reorder(i, half):
            held[half], = reorder_columns([qkv_slab(m, i, half)])
        return [w for i in range(D // 32) for w in (
            functools.partial(reorder, i, 0), functools.partial(reorder, i, 1),
            lambda i=i: qkv_sums(m, i, held[0], held[1]))]

    def prep_wo():
        def staged(e, j, a):
            return 9 * (32 * e + 8 * (j >> 1) + 4 * (j & 1) + a)

        def widen(i):
            j, a = i // 4, i % 4
            seen = []
            for n in range(NL):
                w = wo_raw[32 * i:32 * (i + 1), lanes(n)].astype(F32)
                for e in range(4):
                    g = w[8 * e:8 * e + 8]
                    hb[n, pl.ds(staged(e, j, a), 8), :] = pltpu.roll(g, 8 - j, 0) if j else g
                seen.append(g)
            return total(seen)

        def rows(n, t, e, j_hi):
            return [hb[n, pl.ds(staged(e, 4 * j_hi + 2 * j_mid, 0) + t, 8, stride=9), :]
                    for j_mid in range(2)]

        def sums(n, t, e):
            seen = []
            for j_hi in range(2):
                blk = [rows(n, t, e, j_hi), rows(n + 4, t, e, j_hi),
                       rows(n, t + 4, e, j_hi), rows(n + 4, t + 4, e, j_hi)]
                r = 64 * t + 16 * e + 8 * j_hi
                words = [pack(*rhs_term(p, *blk)) for p in range(7)]
                for p in range(7):
                    wo_c[n * 7 + p, r:r + 8, :] = words[p]
                seen.append(words[5] ^ words[6])
            return seen[0] ^ seen[1]

        return ([functools.partial(widen, i) for i in range(D // 32)]
                + [functools.partial(sums, n, t, e)
                   for n in range(4) for t in range(4) for e in range(4)])

    def prep_ffn(step):
        groups = ((1, 5), (2, 4, 0), (3, 6))

        def piece(load, store, group):
            held = {}

            def block(q):
                if q not in held:
                    held[q] = [x for r in range(2) for c in range(2)
                               for x in unpack(load(2 * (q // 2) + r, 2 * (q % 2) + c))]
                return held[q]
            for p in group:
                o = rhs_term(p, *[block(q) if q in RHS_BLOCKS[p] else None for q in range(4)])
                words = [pack(*rhs_term(j, o[0:2], o[2:4], o[4:6], o[6:8])) for j in range(7)]
                for j in range(7):
                    store(p * 7 + j, words[j])
            return words[2] ^ words[3]

        def up(c, i, n):
            def load(r, b):
                rows = aligned(256 * r + 16 * i, 16)
                return pltpu.bitcast(w1_raw[c + zero[n], rows, lanes(b)], U32)

            def store(p, word):
                w1_c[c, p, aligned(8 * i, 8), :] = word
            return piece(load, store, groups[n])

        def down(c, g, n):
            i, half = g >> 1, g & 1

            def load(r, b):
                return pltpu.bitcast(w2_raw[c + zero[n], aligned(128 * r + 16 * i, 16),
                                            aligned((4 * half + b) * LANE, LANE)], U32)

            def store(p, word):
                w2_c[half, p, c, aligned(8 * i, 8), :] = word
            return piece(load, store, groups[n])

        slabs = [(NC - 1, jnp.minimum(SHARE * step + i, 15)) for i in range(SHARE)]
        slabs += [(step, i) for i in range(16)]
        return [functools.partial(f, c, i, n) for c, i in slabs for f in (up, down)
                for n in range(len(groups))]

    def ln1(t, slot):
        mean, inv = {}, {}

        def load(k, rh, i, cols):
            return pltpu.bitcast(xb[tile_rows(t + zero[k], rh * RA + 16 * i, 16), cols], U32)

        def rows_of(k, rh, i):
            w = load(k, rh, i, slice(None))
            return zip(*[unpack(w[:, lanes(j)]) for j in range(NL)])

        def means(rh, i):
            part = [total(x) for x in rows_of(0, rh, i)]
            mean[rh, i] = [lane_mean(p) for p in part]
            return total(part)

        def scales(rh, i):
            part = [total([(u - m) * (u - m) for u in x])
                    for x, m in zip(rows_of(1, rh, i), mean[rh, i])]
            inv[rh, i] = [jax.lax.rsqrt(lane_mean(p) + EPS) for p in part]
            return total(part)

        def sums(i, j):
            blk = [[(u - m) * r for u, m, r in zip(unpack(load(2, rh, i, lanes(j + 4 * kh))),
                                                   mean[rh, i], inv[rh, i])]
                   for rh in range(2) for kh in range(2)]
            words = [pack(*lhs_term(p, *blk)) for p in range(7)]
            for p in range(7):
                a1[slot, p, 8 * i:8 * i + 8, lanes(j)] = words[p]
            return words[5] ^ words[6]

        groups = [(rh, i) for i in range(RA // 16) for rh in range(2)]
        return ([functools.partial(means, *g) for g in groups],
                [functools.partial(scales, *g) for g in groups],
                [functools.partial(sums, i, j) for i in range(RA // 16) for j in range(4)])

    def project(slot, m, buf, dst, before=None, order=ORDER_PROJ):
        for n in range(4):
            if before:
                before(n)

            def product(p):
                r = mm(as_bf16(a1[slot, p]), as_bf16(wqkv_c[m, n * 7 + p]))
                yield
                return [r]

            def emit(k, c):
                r = HALO + (k // 2) * RA
                buf[dst, n + 4 * (k % 2), r:r + RA, :] = c[0]
            yield from combine(product, emit, order)

    def first_halo():
        for j in range(NL):
            qkv[1, j, 0:HALO, :] = jnp.zeros((HALO, LANE), F32)
            qkv[2, j, 0:HALO, :] = jnp.broadcast_to(qkv[2, j, HALO:HALO + 1, :], (HALO, LANE))

    def hand_over(moved_rows):
        def move(m, r, n):
            for j in range(NL):
                qkv[m, j, HALO + r:HALO + r + n, :] = new[m, j, HALO + r:HALO + r + n, :]
            moved_rows[m] += n
            return qkv[m + zero[7], 0, HALO + r:HALO + r + 8, :]
        for m in (1, 2):
            for j in range(NL):
                qkv[m, j, 0:HALO, :] = qkv[m, j, TM:TM + HALO, :]
            move(m, 0, 16)
        return [[functools.partial(move, m, r, 24) for r in range(16, TM, 24)] for m in (1, 2)]

    def attention(buf, first=False, moved=(True,) * 4):
        held = {}

        def window(r, w):
            return pl.ds(HALO + r - DIL * w, 8)

        def score(r, w):
            if w == 0:
                held[r, "q"] = [(buf if moved[j % 4] else new)[0, j, HALO + r:HALO + r + 8, :]
                                for j in range(NL)]
            a = total([held[r, "q"][j] * buf[1, j, window(r, w), :] for j in range(NL)])
            held[r, w] = a + pltpu.roll(a, 64, 1)

        def logit(r, w):
            a = (held[r, w] + pltpu.roll(held[r, w], 32, 1)) * (DH ** -0.5 * LOG2E)
            if first and r < DIL * w:
                pos = r + jax.lax.broadcasted_iota(I32, (8, LANE), 0)
                a = jnp.where(pos >= DIL * w, a, -1e9 * LOG2E)
            held[r, w] = a
            held[r, "max"] = a if w == 0 else jnp.maximum(held[r, "max"], a)

        def softmax(r):
            ex = [jnp.exp2(held[r, w] - held[r, "max"]) for w in range(WIN)]
            inv = 1.0 / total(ex)
            held[r] = [e * inv for e in ex]

        def value(r, j):
            o = total([held[r][w] * buf[2, j, window(r, w), :] for w in range(WIN)])
            ob[r:r + 8, lanes(j)] = o
            return o

        return [([functools.partial(score, r, w) for w in range(WIN)],
                 [functools.partial(logit, r, w) for w in range(WIN)],
                 functools.partial(softmax, r),
                 [functools.partial(value, r, j) for j in range(NL)]) for r in range(0, TM, 8)]

    def attention_work(pace, att, riders, pattern, lead=True):
        stages = []
        n = len(att)
        placed = [0] * len(riders)
        for u in range(n + 2):
            work = []
            stages.append(work)
            for w in range(WIN):
                k = 0
                for what in pattern:
                    if what == "s" and u < n:
                        work.append(att[u][0][w])
                    if what == "l" and 1 <= u <= n:
                        work.append(att[u - 1][1][w])
                    if what == "v" and (u >= 2 or lead):
                        work.append(pace.tick(att[u - 2][3][w] if u >= 2 else None))
                    if what == "r":
                        thunks, lo, hi = riders[k]
                        want = (WIN * (u - lo) + w + 1) * len(thunks) // (WIN * (hi - lo))
                        want = min(len(thunks), max(0, want))
                        work += thunks[placed[k]:want]
                        placed[k] = want
                        k += 1
            if 1 <= u <= n:
                work.append(att[u - 1][2])
        assert placed == [len(thunks) for thunks, _, _ in riders]
        return stages

    def norm_riders(pace, norm, *bounds):
        return [([pace.tick(w) for w in stage], lo, hi)
                for stage, lo, hi in zip(norm, bounds, bounds[1:])]

    def out_sums():
        def unit(s, i):
            blk = []
            for rh in range(2):
                r = (2 * s + rh) * RO + 16 * i
                blk += [[ob[r:r + 16, lanes(4 * kh, 4)]] for kh in range(2)]
            terms = [lhs_term(p, *blk)[0] for p in range(7)]
            for p in range(7):
                r = (s * 7 + p) * RO + 16 * i
                o_c[r:r + 16, :] = terms[p].astype(BF16)
            return terms[5][0:8, lanes(0)] + terms[6][8:16, lanes(3)]
        return [functools.partial(unit, s, i) for s in range(2) for i in range(RO // 16)]

    def out_proj(t, halves, order):
        for s in halves:
            for n in range(4):
                def product(p):
                    r = mm(o_c[(s * 7 + p) * RO:(s * 7 + p + 1) * RO, :], as_bf16(wo_c[n * 7 + p]))
                    yield
                    return [r]

                def emit(k, c):
                    r = tile_rows(t, (2 * s + k // 2) * RO, RO)
                    j = n + 4 * (k % 2)
                    hb[j, r, :] = xb[r, lanes(j)].astype(F32) + c[0]
                yield from combine(product, emit, order)

    def quad_rows(t, rb, i):
        return tile_rows(t, rb * RB + 32 * (i % 2) + i // 2, 8, stride=4)

    def ln2_stats(t):
        def means(rb, i):
            part = total([hb[j, quad_rows(t, rb, i), :] for j in range(NL)])
            stats[0, tile_rows(t, rb * RB + 8 * i, 8), :] = jnp.broadcast_to(lane_mean(part), (8, LANE))
            return part

        def scales(rb, i):
            dst = tile_rows(t, rb * RB + 8 * i, 8)
            mean = stats[0, dst, :]
            cen = [hb[j, quad_rows(t + zero[6], rb, i), :] - mean for j in range(NL)]
            part = total([u * u for u in cen])
            stats[1, dst, :] = jnp.broadcast_to(0.5 * jax.lax.rsqrt(lane_mean(part) + EPS), (8, LANE))
            return part
        return [functools.partial(f, rb, i) for f in (means, scales) for rb in range(4) for i in range(8)]

    def ln2_sums(t):
        z = zero[1]

        def norm(rb, i):
            src = tile_rows(t, rb * RB + 8 * i, 8)
            mean, inv = stats[0, src, :], stats[1, src, :]
            r = rb * RB + 8 * i
            out = [(hb[j, quad_rows(t, rb, i), :] - mean) * inv for j in range(NL)]
            for j in range(NL):
                zb[z, j, r:r + 8, :] = out[j]
            return total(out)

        def sums(i, n, p):
            blk = [[[zb[zero[2 + p % 4], 2 * c + n, pl.ds(rb * RB + 8 * (i + 4 * h), 8), :]
                     for h in range(2)] for c in range(4)] for rb in range(4)]
            words = [pack(*term) for term in lhs_terms2(blk, p)]
            for j in range(7):
                a2[0, p * 7 + j, 8 * i:8 * i + 8, lanes(n)] = words[j]
            return words[5] ^ words[6]

        return ([functools.partial(norm, rb, i + 4 * h)
                 for i in range(4) for rb in range(4) for h in range(2)]
                + [functools.partial(sums, i, n, p)
                   for i in range(4) for n in range(2) for p in range(7)])

    def ffn_step(t, carry):
        g = [[] for _ in range(49)]
        pace = Pacer(1)
        for c in range(NC):
            act = {}

            def leaf(p):
                r = mm(as_bf16(a2[0, p]), as_bf16(w1_c[c, p]))
                yield
                return [r]

            def emit(rb, nb, v):
                act[rb, nb] = v * jnp.tanh(v) + v
            run(combine2(leaf, emit, ORDER_UP), 49)
            blk = [[[act[rb, nb][:RB // 2], act[rb, nb][RB // 2:]] for nb in range(4)]
                   for rb in range(4)]
            for p in range(7):
                for j, term in enumerate(lhs_terms2(blk, p)):
                    g[p * 7 + j].append(pack(*term))

        def down(n):
            left = [8, 8]

            def leaf(p):
                r = mm(as_bf16(jnp.concatenate(g[p], axis=1)),
                       as_bf16(w2_c[n, p].reshape(F // 8, LANE)))
                yield
                return [r]

            def emit(rb, nb, y):
                r = tile_rows(t, rb * RB, RB)
                xb[r, lanes(4 * n + nb)] = (hb[4 * n + nb, r, :] + y).astype(BF16)
                left[rb // 2] -= 1
                if not left[rb // 2]:
                    cp_y(t, n, rb // 2).start()
            yield from combine2(leaf, emit, ORDER_DOWN)

        sums = ln2_sums(jnp.minimum(t + 1, NT - 1))
        moments = ln2_stats(jnp.minimum(t + 2, NT - 1))
        side = sums[:32] + moments[:32] + sums[32:46] + moments[32:] + sums[46:]
        run(chain(down(0), down(1)), 98, [pace.tick(w) for w in side])
        pace.finish(sink.at[0], 1)
        return carry

    def prologue():
        early = [cp_q(k) for k in range(QPARTS)] + [cp_qkv(1), cp_qkv(2)]

        def start_early(k):
            for i, cp in enumerate(early):
                pl.when(k == i)(cp.start)
        cp_x(0).start()
        cp_x(1).start()

        def first_norm(t, carry):
            start_early(t)
            cp_x(t).wait()
            for stage in ln1(t, t):
                for w in stage:
                    w()
            return carry
        jax.lax.fori_loop(0, 2, first_norm, 0)

        def first_weights(g, carry):
            per_part = D // 32 // 4 // QPARTS

            @pl.when(g % per_part == 0)
            def _():
                start_early(2 + g // per_part)
                cp_q(g // per_part).wait()
            slabs = reorder_columns([qkv_slab(0, 4 * g + i, half)
                                     for i in range(4) for half in range(2)])
            for i in range(4):
                qkv_sums(0, 4 * g + i, slabs[2 * i], slabs[2 * i + 1])
            return carry
        jax.lax.fori_loop(0, D // 32 // 4, first_weights, 0)

        def first_projections(i, carry):
            pl.when(i == 0)(cp_wo().start)
            pl.when(i == 1)(cp_x(2).start)
            pl.when(i == 2)(cp_w1(0).start)
            pl.when(i > 0)(lambda: cp_qkv(jnp.maximum(i, 1)).wait())
            run(project(i & 1, i >> 1, qkv, 3 * (i & 1) + (i >> 1)), N_PROJ, prep_qkv(i))
            return carry
        jax.lax.fori_loop(0, 3, first_projections, 0)

        cp_w2(0).start()
        cp_wo().wait()
        work = prep_wo()
        pace = Pacer(3)
        run(project(0, 2, qkv, 2, order=ORDER_FIRST_V), N_PROJ, [pace.tick(w) for w in work])
        pace.finish(sink.at[1], 1)

        cp_x(3).start()
        cp_w1(NC - 1).start(priority=1)
        cp_w2(NC - 1).start(priority=1)
        cp_x(2).wait()
        first_halo()
        for j in range(NL):
            new[0, j, HALO:, :] = qkv[3, j, HALO:, :]
        pace = Pacer(7)
        norm = norm_riders(pace, ln1(2, 0), 0, 6, 16, 34)
        stages = attention_work(pace, attention(qkv, True), [norm[1], norm[0], norm[2]], "svlrrr")
        run(chain(project(1, 1, new, 1), project(1, 2, new, 2)), 2 * N_PROJ, sum(stages, []))
        pace.finish(sink.at[4], 0)
        cp_w1(NC - 1).wait()
        cp_w2(NC - 1).wait()

    def attention_step(t, carry):
        pl.when(t + 3 < NT)(lambda: cp_x(jnp.minimum(t + 3, NT - 1)).start())

        @pl.when(t < NC - 1)
        def _():
            cp_w1(t).start()
            cp_w2(t).start()
        cp_w1(t - 1).wait()
        cp_w2(t - 1).wait()
        pl.when(t + 2 < NT)(lambda: cp_x(jnp.minimum(t + 2, NT - 1)).wait())

        pace = Pacer(5)
        cut = 24
        moved_rows = [0, 0, 0]
        keys, values = hand_over(moved_rows)
        norm = norm_riders(pace, ln1(jnp.minimum(t + 2, NT - 1), 0), 8, 16, cut, 34)
        riders = [([pace.tick(w) for w in keys], 0, 7),
                  norm[1],
                  ([w for p in prep_ffn(t - 1) for w in (pace.tick(p), pace.tick())], 0, 29),
                  norm[0],
                  norm[2],
                  ([pace.tick(w) for w in values], 0, 14),
                  ([pace.tick(w) for w in out_sums()], 0, 4)]
        moved = [False] * 4

        def move_queries(n):
            for j in (n, n + 4):
                qkv[0, j, HALO:, :] = new[0, j, HALO:, :]
            moved[n] = True

        def check(m):
            def before(n):
                assert moved_rows[m] == TM
            return before
        stages = attention_work(pace, attention(qkv, moved=moved), riders, "slvrrrrrrr")
        run(chain(project(0, 0, new, 0, move_queries, ORDER_STEP[0]),
                  project(0, 1, new, 1, check(1), ORDER_STEP[1]),
                  project(0, 2, new, 2, check(2), ORDER_STEP[2])),
            3 * N_PROJ, sum(stages[:cut], []))
        run(out_proj(t - 1, (0, 1), ORDER_PROJ), 2 * N_PROJ, sum(stages[cut:], []))
        pace.finish(sink.at[2], 1)
        return carry

    def epilogue():
        for m in (1, 2):
            for j in range(NL):
                new[m, j, 0:HALO, :] = qkv[m, j, TM:TM + HALO, :]
        for w in out_sums():
            w()
        pace = Pacer(11)
        norm = [pace.tick(w) for w in ln2_stats(0) + ln2_sums(0) + ln2_stats(1)]
        few = len(norm) // 5
        sums = out_sums()
        stages = attention_work(pace, attention(new),
                                [(norm[:few], 26, 34), (sums[:len(sums) // 2], 18, 19)],
                                "lrvsr", False)
        run(out_proj(NT - 2, (0, 1), ORDER_LAST[0]), 2 * N_PROJ, sum(stages[:19], []))
        run(out_proj(NT - 1, (0,), ORDER_LAST[1]), N_PROJ,
            sum(stages[19:], []) + sums[len(sums) // 2:])
        run(out_proj(NT - 1, (1,), ORDER_LAST[2]), N_PROJ, norm[few:])
        pace.finish(sink.at[3], 0)

    prologue()
    jax.lax.fori_loop(1, NT - 1, attention_step, 0)
    epilogue()
    jax.lax.fori_loop(0, NT, ffn_step, 0)
    for t in range(NT):
        for k in range(4):
            cp_y(t, k // 2, k % 2).wait()


@jax.jit
def pallas_sequential_preLN__sliding_local_dilated__dense_activation_silu__prompt_kernel(
    A_x: jax.Array,
    A_wqkv: jax.Array,
    A_wo: jax.Array,
    B_x: jax.Array,
    B_w1: jax.Array,
    B_w2: jax.Array,
):
    del B_x
    vmem = pltpu.VMEM
    dma = pltpu.SemaphoreType.DMA
    hbm = pl.BlockSpec(memory_space=pl.ANY)
    out = pl.pallas_call(
        kernel,
        in_specs=[hbm] * 5,
        out_specs=hbm,
        out_shape=jax.ShapeDtypeStruct((S, D), BF16),
        scratch_shapes=[
            vmem((S, D), BF16),
            vmem((2, D // 2, 3 * D), BF16), vmem((D, D), BF16),
            vmem((NC, D, FC), BF16), vmem((NC, FC, D), BF16),
            vmem((3, 4 * 7, D // 4, LANE), U32),
            vmem((4 * 7, D // 4, LANE), U32),
            vmem((NC, 49, D // 8, LANE), U32),
            vmem((2, 49, NC, FC // 8, LANE), U32),
            vmem((2, 7, RA // 2, D // 2), U32),
            vmem((4, NL, TM + HALO, LANE), F32),
            vmem((3, NL, TM + HALO, LANE), F32),
            vmem((TM, D), F32), vmem((7 * TM // 2, D // 2), BF16),
            vmem((NL, S + 8, LANE), F32),
            vmem((2, S, LANE), F32), vmem((1, NL, TM, LANE), F32),
            vmem((1, 49, RB // 2, D // 4), U32),
            vmem((5, 8, LANE), F32), pltpu.SMEM((8,), I32),
            dma((NT,)), dma((3 + QPARTS,)), dma((NC,)), dma((NC,)), dma((4 * NT,)),
        ],
        compiler_params=pltpu.CompilerParams(vmem_limit_bytes=126 * 2 ** 20,
                                             disable_bounds_checks=True),
    )(A_x.reshape(S, D), A_wqkv.reshape(2, D // 2, 3 * D), A_wo, B_w1, B_w2)
    return out.reshape(1, S, D)
```
